```python
import os as _os
_os.environ.setdefault("JAX_PLATFORMS", "cpu")
import jax
import jax.numpy as jnp

def _softmax(x, axis=-1):
    return jax.nn.softmax(x, axis=axis)
def _gelu(x):
    return jax.nn.gelu(x, approximate=True)
def _silu(x):
    return jax.nn.silu(x)
def _sigmoid(x):
    return jax.nn.sigmoid(x)
def _layernorm(x, axis=-1, eps=1e-5):
    m = jnp.mean(x, axis=axis, keepdims=True)
    v = jnp.var(x, axis=axis, keepdims=True)
    return (x - m) / jnp.sqrt(v + eps)
def _scatter_add(tgt, idx, src, axis=0):
    return tgt.at[idx].add(src)
def _segment_sum(src, seg, n):
    return jax.ops.segment_sum(src, seg, n)
class _Rng:
    def __init__(self, key):
        self._k = key
    def _next(self):
        self._k, sub = jax.random.split(self._k)
        return sub
    def normal(self, shape):
        return jax.random.normal(self._next(), shape, dtype=jnp.bfloat16)
    def randint(self, lo, hi, shape):
        return jax.random.randint(self._next(), shape, lo, hi, dtype=jnp.int32)
    def uniform(self, shape, lo=0.0, hi=1.0):
        return jax.random.uniform(self._next(), shape, jnp.bfloat16, lo, hi)
    def permutation(self, n):
        return jax.random.permutation(self._next(), n)


kernel_name = 'concat_heads__ssm_conv_s4__grouped_kv_mqa__prompt'

def setup_inputs():
    _rng = _Rng(jax.random.key(int.from_bytes(__import__("os").urandom(4), "little")))
    _w = (lambda a: (lambda t: t.astype(jnp.bfloat16) if jnp.issubdtype(t.dtype, jnp.floating) else t)(jnp.asarray(a)))
    def _A_setup():
        B, L, D, N = 1, 2048, 448, 256
        A_re = -jnp.exp((lambda *s: _rng.normal(s) * 0.1)(D, N))
        A_im = jnp.pi * (lambda *s: _rng.normal(s) * 0.1)(D, N)
        B_re = (lambda *s: _rng.normal(s) * 0.1)(D, N)
        B_im = (lambda *s: _rng.normal(s) * 0.1)(D, N)
        C_re = (lambda *s: _rng.normal(s) * 0.1)(D, N)
        C_im = (lambda *s: _rng.normal(s) * 0.1)(D, N)
        log_dt = (lambda *s: _rng.normal(s) * 0.1)(D) * 0.5 - 4.0
        Dskip = (lambda *s: _rng.normal(s) * 0.05)(D)
        return {
            "u": _w((lambda *s: _rng.normal(s) * 0.05)(B, L, D)),
            "A_re": _w(A_re),
            "A_im": _w(A_im),
            "B_re": _w(B_re),
            "B_im": _w(B_im),
            "C_re": _w(C_re),
            "C_im": _w(C_im),
            "log_dt": _w(log_dt),
            "Dskip": _w(Dskip),
        }
    _A_in = _A_setup()

    def _B_setup():
        B, S, D, H = 1, 2048, 448, 16
        Dh = D // H
        return {
            "x": _w((lambda *s: _rng.normal(s) * 0.05)(B, S, D)),
            "wq": _w((lambda *s: _rng.normal(s) * 0.8)(D, H * Dh)),
            "wk": _w((lambda *s: _rng.normal(s) * 0.8)(D, Dh)),
            "wv": _w((lambda *s: _rng.normal(s) * 0.05)(D, Dh)),
            "wo": _w((lambda *s: _rng.normal(s) * 0.05)(H * Dh, D)),
        }
    _B_in = _B_setup()

    return {
        "A_u": _A_in["u"],
        "A_A_re": _A_in["A_re"],
        "A_A_im": _A_in["A_im"],
        "A_B_re": _A_in["B_re"],
        "A_B_im": _A_in["B_im"],
        "A_C_re": _A_in["C_re"],
        "A_C_im": _A_in["C_im"],
        "A_log_dt": _A_in["log_dt"],
        "A_Dskip": _A_in["Dskip"],
        "B_x": _B_in["x"],
        "B_wq": _B_in["wq"],
        "B_wk": _B_in["wk"],
        "B_wv": _B_in["wv"],
        "B_wo": _B_in["wo"],
    }

def reference(A_u, A_A_re, A_A_im, A_B_re, A_B_im, A_C_re, A_C_im, A_log_dt, A_Dskip, B_x, B_wq, B_wk, B_wv, B_wo):
    def _A_ref(u, A_re, A_im, B_re, B_im, C_re, C_im, log_dt, Dskip):
        Bsz, L, D = u.shape
        dt = jnp.exp(log_dt)[:, None]
        A = A_re + 1j * A_im
        Bc = B_re + 1j * B_im
        Cc = C_re + 1j * C_im
        logdA = dt * A
        dB = dt * Bc
        l = (lambda x, dt: x.astype(dt))(jnp.arange(L), A_re.dtype)
        P = jnp.exp(logdA[:, :, None] * l[None, None, :])
        K = jnp.einsum("dn,dnl,dn->dl", Cc, P, dB).real
        L2 = 2 * L
        Kp = jnp.pad(K, ((0, 0), (0, L)))
        up = (lambda x, *d: x.transpose(*d))(u, 0, 2, 1)
        up = jnp.pad(up, ((0, 0), (0, 0), (0, L)))
        Kf = (lambda x, axes=(-2,-1): jnp.fft.rfft2(x.astype(jnp.float32), axes=axes))(Kp[:, None, :], axes=(-2, -1))
        Uf = (lambda x, axes=(-2,-1): jnp.fft.rfft2(x.astype(jnp.float32), axes=axes))(up[:, :, None, :], axes=(-2, -1))
        Yf = Uf * Kf[None, :, :, :]
        y = (lambda x, s, axes=(-2,-1): jnp.fft.irfft2(x, s=s, axes=axes).astype(jnp.bfloat16))(Yf, (1, L2), axes=(-2, -1))[:, :, 0, :L]
        y = (lambda x, *d: x.transpose(*d))(y, 0, 2, 1) + u * Dskip[None, None, :]
        return y

    def _B_ref(x, wq, wk, wv, wo):
        B, S, D = x.shape
        H = 16
        Dh = D // H
        q = (lambda x, *d: x.transpose(*d))((x @ wq).reshape(B, S, H, Dh), 0, 2, 1, 3)
        k = x @ wk
        v = x @ wv
        scores = jnp.einsum("bhqd,bkd->bhqk", q, k) * (Dh ** -0.5)
        p = _softmax(scores, axis=-1)
        o = jnp.einsum("bhqk,bkd->bhqd", p, v)
        return (lambda x, *d: x.transpose(*d))(o, 0, 2, 1, 3).reshape(B, S, H * Dh) @ wo

    a = _A_ref(A_u, A_A_re, A_A_im, A_B_re, A_B_im, A_C_re, A_C_im, A_log_dt, A_Dskip)
    b = _B_ref(B_x, B_wq, B_wk, B_wv, B_wo)
    return jnp.concatenate([a, b], axis=-1)
```

```python
import numpy as np

import jax
import jax.numpy as jnp
import jax.experimental.pallas as pl
import jax.experimental.pallas.tpu as pltpu

F32 = jnp.float32
BF16 = jnp.bfloat16

L = 2048
D = 448
N = 256
H = 16
DH = D // H
DP = 32
T = 128
NC = L // T
QW = 512
NQB = L // QW
NU = NQB * H
KB = 128
CG = 8
NG = D // CG
G = 4

TAP_STEPS = (
    (6, 8, 9, 10, 11, 12, 13, 14),
    (7, 8, 9, 10, 11, 12, 13, 14),
    (7, 8, 9, 10, 11, 12, 13, 14),
    (7, 8, 9, 10, 11, 12, 13, 14),
)
CONV_STEPS = ((2, 14), (1, 14), (1, 14), (1, 15))
TABLE_STEPS = ((0, 1, 2), (0, 3, 5), (0, 3, 5), (1, 3, 5))
OUT_STEPS = (-1, 1, 1, 2, 3, 4, 6, 7, 8, 10, 11, 13)


def _dft_matrices():
    t = np.arange(T, dtype=np.float64)[:, None]
    f = np.arange(T, dtype=np.float64)[None, :]
    ang = np.pi * (2.0 * f + 1.0) * t / (2.0 * T)
    fwd = np.concatenate([np.cos(ang), -np.sin(ang)], axis=1)
    inv = np.concatenate([np.cos(ang.T), -np.sin(ang.T)], axis=0) / T
    col = np.arange(T)
    fwd = np.stack([fwd, fwd[16 * (col % 8) + col // 8]])
    return _pack_rows(fwd), _pack_rows(inv)


def _pack_rows(a):
    bits = a.astype(np.float32).view(np.uint32)
    bits = (bits + 0x7FFF + ((bits >> 16) & 1)) >> 16
    return (bits[..., 0::2, :] | (bits[..., 1::2, :] << 16)).astype(np.uint32)


_FWD_NP, _INV_NP = _dft_matrices()


def _cmul(ar, ai, br, bi):
    return ar * br - ai * bi, ar * bi + ai * br


def _dot(a, b):
    return jnp.dot(a, b, preferred_element_type=F32)


def _pack(a):
    return pltpu.bitcast(a, jnp.uint32)


def _unpack(a):
    return pltpu.bitcast(a, BF16)


def _fold_bits(a):
    bits = pltpu.bitcast(a, jnp.uint32)
    out = None
    for r in range(0, a.shape[0], 8):
        for c in range(0, a.shape[1], 128):
            tile = bits[r:r + 8, c:c + 128]
            out = tile if out is None else out | tile
    return out


def _after(a, bits, zero):
    head = _pack(a[:16, :128]) | (bits & zero)
    head = jnp.concatenate([_unpack(head), a[:16, 128:]], axis=1)
    return jnp.concatenate([head, a[16:]], axis=0)


def _aligned(i, n):
    return i if isinstance(i, int) else pl.multiple_of(i, n)


def _column(vec_ref):
    row = vec_ref[...].astype(F32).reshape(1, D)
    row = jnp.concatenate([row, jnp.zeros((1, 512 - D), F32)], axis=1)
    return jnp.broadcast_to(row, (128, 512)).T[:D]


def _kernel(
    ut_hbm, are_hbm, aim_hbm, bre_hbm, bim_hbm, cre_hbm, cim_hbm, ldt_hbm, dsk_hbm,
    xt_hbm, wq_hbm, wkt_hbm, wvt_hbm, wo_hbm, fwd_hbm, inv_hbm,
    out_hbm,
    ut_v, par_v, ldt_v, dsk_v, xt_v, wq_v, wkt_v, wvt_v, wo_v, dft_v, inv_v,
    lam_s, c_s, dsk_s, dt_s, wt_s, wot_s, q_s, k_s, vt_s, s_s, o_s, y_s,
    pow_s, w_s, kt_s, m_s, out_v, in_sem, x_sem, out_sem,
):
    copies = {}

    def start(name, src, dst):
        cp = pltpu.make_async_copy(src, dst, in_sem.at[len(copies)])
        cp.start()
        copies[name] = cp

    def x_copy(j):
        cols = pl.ds(_aligned(j * QW, QW), QW)
        return pltpu.make_async_copy(xt_hbm.at[:, cols], xt_v.at[:, cols], x_sem.at[j])

    start("ldt", ldt_hbm, ldt_v)
    start("dsk", dsk_hbm, dsk_v)
    start("wq", wq_hbm, wq_v)
    start("wk", wkt_hbm, wkt_v)
    start("wv", wvt_hbm, wvt_v)
    x_copy(0).start()
    copies["ldt"].wait()
    copies["dsk"].wait()
    dt_s[...] = jnp.exp(_column(ldt_v)).astype(BF16).astype(F32)
    dsk_s[...] = _column(dsk_v)

    for name in ("wq", "wk", "wv"):
        copies[name].wait()
    x_copy(1).start()
    wq = jnp.concatenate([wq_v[...], jnp.zeros((D, 512 - D), BF16)], axis=1)
    wq = jnp.concatenate([wq, jnp.zeros((512 - D, 512), BF16)], axis=0)
    wt_s[0:D, :] = wq.T[:D, :D]
    zpad = jnp.zeros((DP - DH, D), F32)
    wt_s[D:D + DP, :] = jnp.concatenate([wkt_v[...].astype(F32), zpad], axis=0).astype(BF16)
    wt_s[D + DP:D + 2 * DP, :] = jnp.concatenate([wvt_v[...].astype(F32), zpad], axis=0).astype(BF16)

    def decay(block, half):
        rows = pl.ds(_aligned(block * 16, 16), 16)
        cols = pl.ds(half * 128, 128)
        dt = dt_s[rows, :]
        mag = jnp.exp(dt * par_v[0, rows, cols].astype(F32))
        ang = dt * par_v[1, rows, cols].astype(F32)
        x, y = mag * jnp.cos(ang), mag * jnp.sin(ang)
        lam_s[0, rows, cols] = x
        lam_s[1, rows, cols] = y
        return _fold_bits(x) | _fold_bits(y)

    qscale = float(DH ** -0.5 * np.log2(np.e))
    row = jax.lax.broadcasted_iota(jnp.int32, (DP, QW), 0)
    later = [(ref, par_v.at[i]) for i, ref in enumerate((are_hbm, aim_hbm, bre_hbm, bim_hbm, cre_hbm, cim_hbm))]
    later += [(wo_hbm, wo_v), (ut_hbm, ut_v), (fwd_hbm, dft_v), (inv_hbm, inv_v)]
    later = [pltpu.make_async_copy(src, dst, in_sem.at[len(copies) + i]) for i, (src, dst) in enumerate(later)]

    def project(j, carry):
        x_copy(j).wait()

        @pl.when(j < NQB - 2)
        def _():
            x_copy(j + 2).start()

        @pl.when(j == 2)
        def _():
            for cp in later[:7]:
                cp.start()

        cols = pl.ds(pl.multiple_of(j * QW, QW), QW)
        x = xt_v[:, cols]
        kv = _dot(wt_s[D:D + 2 * DP, :], x)
        kt = jnp.concatenate([kv[:DP], jnp.zeros((128 - DP, QW), F32)], axis=0)
        k_s[pl.ds(pl.multiple_of(j * (QW // 2), QW // 2), QW // 2), :] = _pack(kt.T[:, :DP].astype(BF16))
        vt_s[:, cols] = _pack(jnp.where(row == DH, 1.0, kv[DP:]).astype(BF16))
        for t in range(4):
            q4 = _dot(wt_s[4 * t * DH:4 * (t + 1) * DH, :], x)
            q4 = jnp.concatenate([q4, jnp.zeros((8, QW), F32)], axis=0)
            for h in range(4):
                qh = q4[h * DH:h * DH + DP] * qscale
                q_s[j * H + 4 * t + h] = jnp.where(row < DH, qh, 0.0).astype(BF16)
        return carry

    jax.lax.fori_loop(0, NQB, project, 0)

    def input_weights(k):
        for r in range(0, D // 4, 16):
            rows = pl.ds(pl.multiple_of(k * (D // 4) + r, 16), 16)
            par = lambda i: par_v[i, rows, :].astype(F32)
            dt = dt_s[rows, :]
            dt = jnp.concatenate([dt, dt], axis=1)
            cr, ci = _cmul(par(4), par(5), dt * par(2), dt * par(3))
            c_s[0, rows, :], c_s[1, rows, :] = cr, ci
        return _fold_bits(ci[:8])

    def out_weights(k):
        wo = wo_v[pl.ds(pl.multiple_of(k * 4 * DH, 16), 4 * DH), :].astype(F32)
        wo = jnp.concatenate([wo, jnp.zeros((4 * DH, 512 - D), F32)], axis=1)
        pieces = []
        for h in range(4):
            pieces += [wo[h * DH:(h + 1) * DH], jnp.zeros((DP - DH, 512), F32)]
        wot = jnp.concatenate(pieces, axis=0).T[:D]
        wot_s[k] = wot.astype(BF16)
        return _fold_bits(wot[D - 8:])

    def drain(gen):
        for _ in gen:
            pass

    lane = jax.lax.broadcasted_iota(jnp.int32, (CG, T), 1)
    sign = jnp.where((lane & 1) == 0, 1.0, -1.0).astype(F32)

    def group_rows(g):
        return pl.ds(_aligned(g * CG, CG), CG)

    def ssm_tables(g, buf):
        rows = group_rows(g)
        x, y = lam_s[0, rows, :], lam_s[1, rows, :]
        y2 = y * y

        def put(ref, part, k, val):
            for half in range(2):
                ref[buf, part, half, k * CG:(k + 1) * CG, :] = val[:, half * 128:(half + 1) * 128]

        def square(t, s):
            return t * t - y2 * (s * s), (t + t) * s

        put(pow_s, 0, 8, x)
        put(pow_s, 1, 8, y2)
        t, s = x * x - y2, x + x
        for _ in range(3):
            t, s = square(t, s)
        pows = [(jnp.ones_like(x), jnp.zeros_like(x)), (t, s)]
        ys = y2 * s
        for k in range(2, 9):
            if k % 2 == 0:
                pows.append(square(*pows[k // 2]))
            else:
                pt, ps = pows[k - 1]
                pows.append((pt * t - ps * ys, pt * s + ps * t))
        for k in range(8):
            put(pow_s, 0, k, pows[k][0])
            put(pow_s, 1, k, pows[k][1])
        yield _fold_bits(pows[7][1])
        pt, ps = pows[8]
        yps = y2 * ps
        wr, wv = c_s[0, rows, :], c_s[1, rows, :] * -y
        for m in range(NC):
            put(w_s, 0, m, wr)
            put(w_s, 1, m, wv)
            if m + 1 < NC:
                wr, wv = wr * pt + wv * ps, wv * pt - wr * yps
            if m % 8 == 7:
                yield _fold_bits(wv)

    def ssm_taps(buf):
        def powers(c):
            tiles = []
            for half in range(2):
                t = pow_s[buf, 0, half, pl.ds(c, 8, stride=CG), :]
                s = pow_s[buf, 1, half, pl.ds(c, 8, stride=CG), :]
                mx = jnp.broadcast_to(pow_s[buf, 0, half, pl.ds(8 * CG + c, 1), :], (8, 128))
                my = jnp.broadcast_to(pow_s[buf, 1, half, pl.ds(8 * CG + c, 1), :], (8, 128))
                tt, ts = [t], [s]
                for _ in range(T // 8 - 1):
                    t, s = mx * t - my * s, mx * s + t
                    tt.append(t)
                    ts.append(s)
                tiles += [(part, half, _pack(jnp.concatenate(tab, axis=0).astype(BF16).T))
                          for part, tab in enumerate((tt, ts))]
            return tiles

        for c in range(CG):
            acc = None
            for part, half, tab in powers(c):
                w = w_s[buf, part, half, pl.ds(c, NC, stride=CG), :].astype(BF16)
                d = _dot(w, _unpack(tab))
                acc = d if acc is None else acc + d
            kt_s[buf, pl.ds(c, NC, stride=CG), :] = acc
            yield

    def ssm_conv(g, odd, buf):
        rows = group_rows(g)
        kt = kt_s[buf, 0:NC * CG, :]
        kf = _dot(kt.astype(BF16), _unpack(dft_v[1]))
        pair = pl.ds(_aligned((g // 2) * (2 * CG), 2 * CG), 2 * CG)
        load_u = lambda j: ut_v[pair, j * T:(j + 1) * T].astype(F32)[odd * CG:(odd + 1) * CG]
        u = jnp.concatenate([load_u(j) for j in range(NC)], axis=0)
        uf = _dot(u.astype(BF16), _unpack(dft_v[0]))
        yield
        blk = lambda a, j, p: a[j * CG:(j + 1) * CG, p * T:(p + 1) * T]
        gr, gs, gd, us, zs = [], [], [], [], []
        for i in range(NC):
            re, im = blk(kf, i, 0), blk(kf, i, 1)
            if i > 0:
                re, im = re - sign * blk(kf, i - 1, 1), im + sign * blk(kf, i - 1, 0)
            gr.append(re)
            gs.append(re + im)
            gd.append(im - re)
            us.append(blk(uf, i, 0) + blk(uf, i, 1))
            k1 = k2 = k3 = None
            for j in range(i + 1):
                t1, t2, t3 = gr[i - j] * us[j], gs[i - j] * blk(uf, j, 1), gd[i - j] * blk(uf, j, 0)
                k1 = t1 if k1 is None else k1 + t1
                k2 = t2 if k2 is None else k2 + t2
                k3 = t3 if k3 is None else k3 + t3
            zs.append(jnp.concatenate([k1 - k2, k1 + k3], axis=1))
        y = _dot(jnp.concatenate(zs, axis=0).astype(BF16), _unpack(inv_v[...]))
        dsk = dsk_s[rows, :]
        for j in range(NC):
            y_s[rows, j * T:(j + 1) * T] = y[j * CG:(j + 1) * CG] + dsk * load_u(j)
        yield

    def runtime_zero(i):
        return jnp.full((8, 128), i // NU, jnp.int32).astype(jnp.uint32)

    def scores(q, slot, j):
        r = pl.ds(j * KB, KB)
        s = _dot(_unpack(k_s[pl.ds(j * KB // 2, KB // 2), :]), q)
        s_s[slot, r, :] = s
        return jnp.max(s.reshape(KB // 8, 8, QW), axis=0)

    def attn_step(i, slot, with_scores, side):
        if with_scores:
            q = q_s[i + G]
            zero = runtime_zero(i)
        m_cur = m_s[slot]
        mx = acc = None
        for j in range(L // KB):
            r = pl.ds(j * KB, KB)
            p = jnp.exp2(s_s[slot, r, :] - m_cur).astype(BF16)
            d = _dot(_unpack(vt_s[:, r]), p)
            acc = d if acc is None else acc + d
            if with_scores:
                t = scores(q, slot, j)
                mx = t if mx is None else jnp.maximum(mx, t)
            bits = next(side, None)
            if bits is not None:
                q = _after(q, bits, zero)
        o_s[i] = (acc * (1.0 / acc[DH:DH + 1, :])).astype(BF16)
        if with_scores:
            m_s[slot] = jnp.max(mx, axis=0, keepdims=True)

    def tile_rows(c):
        return pl.ds(_aligned(c * 128, 128), 128)

    def out_copy(c):
        rows = tile_rows(c)
        return pltpu.make_async_copy(out_v.at[rows, :], out_hbm.at[rows, :], out_sem.at[c])

    def out_tile(c):
        rows = tile_rows(c)

        def put(t, val):
            out_v[rows, t * 128:(t + 1) * 128] = val.T.astype(BF16)

        for t in range(3):
            put(t, y_s[t * 128:(t + 1) * 128, rows])
        first = (c // (QW // 128)) * H
        cols = tile_rows(c % (QW // 128))
        ot = o_s[pl.ds(first, H), :, cols].reshape(H * DP, 128)
        for t, lo, hi in ((3, 320, D), (2, 192, 320), (1, 64, 192), (0, 0, 64)):
            w = jnp.concatenate([wot_s[k, lo:hi, :] for k in range(4)], axis=1)
            val = _dot(w, ot)
            if t == 0:
                val = jnp.concatenate([y_s[384:D, rows], val], axis=0)
            put(3 + t, val)
            yield

    for cp in later[:7]:
        cp.wait()

    for cp in later[7:]:
        cp.start()

    def first_scores(k, carry):
        zero = runtime_zero(k)
        q = q_s[k]
        mx = None
        for j in range(L // KB):
            t = scores(q, k, j)
            mx = t if mx is None else jnp.maximum(mx, t)
            if j < 14:
                q = _after(q, decay(7 * k + j // 2, j % 2), zero)
            elif j == 14:
                q = _after(q, input_weights(k) | out_weights(k), zero)
        m_s[k] = jnp.max(mx, axis=0, keepdims=True)
        return carry

    jax.lax.fori_loop(0, G, first_scores, 0)
    for cp in later[7:]:
        cp.wait()

    def main_body(i, carry):
        nxt = G * jnp.minimum(i + 1, NG // G - 1)

        def side():
            tables = ssm_tables(G * i + G - 1, G - 1)
            for k in range(G):
                group = jnp.maximum(G * i + k - 1, 0)
                gens = ((ssm_taps(k), TAP_STEPS[k]),
                        (ssm_conv(group, (k + 1) % 2, (k - 1) % G), CONV_STEPS[k]),
                        (tables, TABLE_STEPS[k]))
                for step in range(L // KB):
                    bits = None
                    for gen, steps in gens:
                        for _ in range(steps.count(step)):
                            new = next(gen, None)
                            if new is not None:
                                bits = new if bits is None else bits | new
                    yield bits
                for gen, _ in gens:
                    drain(gen)
                tables = ssm_tables(nxt + k, k)

        work = side()
        for slot in range(G):
            attn_step(G * i + slot, slot, True, work)
        drain(work)
        return carry

    for k in range(G - 1):
        drain(ssm_tables(k, k))
    kt_s[G - 1, 0:NC * CG, :] = jnp.zeros((NC * CG, T), F32)
    jax.lax.fori_loop(0, NG // G, main_body, 0)
    drain(ssm_conv(NG - 1, 1, G - 1))

    def plain_body(k, carry):
        attn_step(NG + k, k, True, iter(()))
        return carry

    jax.lax.fori_loop(0, G, plain_body, 0)

    def tail_body(k, carry):
        todo = [3 * k + t for t in range(3)]
        pieces = (None for c in todo for _ in out_tile(c))

        def side():
            for step in range(L // KB):
                for _ in range(OUT_STEPS.count(step)):
                    next(pieces)
                yield

        for _ in range(OUT_STEPS.count(-1)):
            next(pieces)
        attn_step(NU - G + k, k, False, side())
        drain(pieces)
        for c in todo:
            out_copy(c).start()
        return carry

    jax.lax.fori_loop(0, G, tail_body, 0)
    for c in range(12, L // 128):
        drain(out_tile(c))
        out_copy(c).start()
    for c in range(L // 128):
        out_copy(c).wait()


@jax.jit
def pallas_concat_heads__ssm_conv_s4__grouped_kv_mqa__prompt_kernel(
    A_u: jax.Array,
    A_A_re: jax.Array,
    A_A_im: jax.Array,
    A_B_re: jax.Array,
    A_B_im: jax.Array,
    A_C_re: jax.Array,
    A_C_im: jax.Array,
    A_log_dt: jax.Array,
    A_Dskip: jax.Array,
    B_x: jax.Array,
    B_wq: jax.Array,
    B_wk: jax.Array,
    B_wv: jax.Array,
    B_wo: jax.Array,
):
    vmem = pltpu.VMEM
    scratch = [
        vmem((D, L), BF16),
        vmem((6, D, N), BF16),
        vmem((D,), BF16),
        vmem((D,), BF16),
        vmem((D, L), BF16),
        vmem((D, D), BF16),
        vmem((DH, D), BF16),
        vmem((DH, D), BF16),
        vmem((D, D), BF16),
        vmem((2, T // 2, 2 * T), jnp.uint32),
        vmem((T, T), jnp.uint32),
        vmem((2, D, N), F32),
        vmem((2, D, N), F32),
        vmem((D, 128), F32),
        vmem((D, 128), F32),
        vmem((D + 2 * DP, D), BF16),
        vmem((4, D, 128), BF16),
        vmem((NU, DP, QW), BF16),
        vmem((L // 2, DP), jnp.uint32),
        vmem((DP // 2, L), jnp.uint32),
        vmem((G, L, QW), F32),
        vmem((NU, DP, QW), BF16),
        vmem((D, L), F32),
        vmem((G, 2, 2, 9 * CG, 128), F32),
        vmem((G, 2, 2, (NC + 1) * CG, 128), F32),
        vmem((G, (NC + 1) * CG, T), F32),
        vmem((G, 1, QW), F32),
        vmem((L, 2 * D), BF16),
        pltpu.SemaphoreType.DMA((16,)),
        pltpu.SemaphoreType.DMA((NQB,)),
        pltpu.SemaphoreType.DMA((L // 128,)),
    ]
    out = pl.pallas_call(
        _kernel,
        out_shape=jax.ShapeDtypeStruct((L, 2 * D), BF16),
        in_specs=[pl.BlockSpec(memory_space=pl.ANY)] * 16,
        out_specs=pl.BlockSpec(memory_space=pl.ANY),
        scratch_shapes=scratch,
        compiler_params=pltpu.CompilerParams(vmem_limit_bytes=100 * 1024 * 1024),
    )(
        A_u[0].T, A_A_re, A_A_im, A_B_re, A_B_im, A_C_re, A_C_im, A_log_dt, A_Dskip,
        B_x[0].T, B_wq, B_wk.T, B_wv.T, B_wo,
        _FWD_NP, _INV_NP,
    )
    return out[None]
```
